```python
import os as _os
_os.environ.setdefault("JAX_PLATFORMS", "cpu")
import jax
import jax.numpy as jnp

def _softmax(x, axis=-1):
    return jax.nn.softmax(x, axis=axis)
def _gelu(x):
    return jax.nn.gelu(x, approximate=True)
def _silu(x):
    return jax.nn.silu(x)
def _sigmoid(x):
    return jax.nn.sigmoid(x)
def _layernorm(x, axis=-1, eps=1e-5):
    m = jnp.mean(x, axis=axis, keepdims=True)
    v = jnp.var(x, axis=axis, keepdims=True)
    return (x - m) / jnp.sqrt(v + eps)
def _scatter_add(tgt, idx, src, axis=0):
    return tgt.at[idx].add(src)
def _segment_sum(src, seg, n):
    return jax.ops.segment_sum(src, seg, n)
class _Rng:
    def __init__(self, key):
        self._k = key
    def _next(self):
        self._k, sub = jax.random.split(self._k)
        return sub
    def normal(self, shape):
        return jax.random.normal(self._next(), shape, dtype=jnp.bfloat16)
    def randint(self, lo, hi, shape):
        return jax.random.randint(self._next(), shape, lo, hi, dtype=jnp.int32)
    def uniform(self, shape, lo=0.0, hi=1.0):
        return jax.random.uniform(self._next(), shape, jnp.bfloat16, lo, hi)
    def permutation(self, n):
        return jax.random.permutation(self._next(), n)


kernel_name = 'sequential_preLN__linear_kernel_hedgehog__geglu_ffn__prompt'

def setup_inputs():
    _rng = _Rng(jax.random.key(int.from_bytes(__import__("os").urandom(4), "little")))
    _w = (lambda a: (lambda t: t.astype(jnp.bfloat16) if jnp.issubdtype(t.dtype, jnp.floating) else t)(jnp.asarray(a)))
    def _A_setup():
        B, S, D, H = 1, 2048, 640, 32
        Dh = D // H
        return {
            "x": _w((lambda *s: _rng.normal(s) * 0.05)(B, S, D)),
            "wqkv": _w((lambda *s: _rng.normal(s) * 0.2)(D, 3 * D)),
            "w_phi": _w((lambda *s: _rng.normal(s) * 0.2)(H, Dh, Dh) * (Dh ** -0.5)),
            "wo": _w((lambda *s: _rng.normal(s) * 0.05)(D, D)),
        }
    _A_in = _A_setup()

    def _B_setup():
        B, S, D, F = 1, 2048, 640, 1536
        return {
            "x": _w((lambda *s: _rng.normal(s) * 0.05)(B, S, D)),
            "w_gate": _w((lambda *s: _rng.normal(s) * 0.05)(D, F)),
            "w_up": _w((lambda *s: _rng.normal(s) * 0.05)(D, F)),
            "w_down": _w((lambda *s: _rng.normal(s) * 0.05)(F, D)),
        }
    _B_in = _B_setup()

    return {
        "A_x": _A_in["x"],
        "A_wqkv": _A_in["wqkv"],
        "A_w_phi": _A_in["w_phi"],
        "A_wo": _A_in["wo"],
        "B_x": _B_in["x"],
        "B_w_gate": _B_in["w_gate"],
        "B_w_up": _B_in["w_up"],
        "B_w_down": _B_in["w_down"],
    }

def reference(A_x, A_wqkv, A_w_phi, A_wo, B_x, B_w_gate, B_w_up, B_w_down):
    def _A_ref(x, wqkv, w_phi, wo):
        B, S, D = x.shape
        H = 32; Dh = D // H
        qkv = (lambda x, *d: x.transpose(*d))((x @ wqkv).reshape(B, S, 3, H, Dh), 2, 0, 3, 1, 4)
        q, k, v = qkv[0], qkv[1], qkv[2]
        pq = jnp.einsum("bhsd,hdf->bhsf", q, w_phi)
        pk = jnp.einsum("bhsd,hdf->bhsf", k, w_phi)
        phi_q = jnp.concatenate([_softmax(pq, axis=-1), _softmax(-pq, axis=-1)], axis=-1)
        phi_k = jnp.concatenate([_softmax(pk, axis=-1), _softmax(-pk, axis=-1)], axis=-1)
        kv = jnp.einsum("bhsf,bhsd->bhfd", phi_k, v)
        z  = jnp.einsum("bhsf->bhf", phi_k)
        num = jnp.einsum("bhqf,bhfd->bhqd", phi_q, kv)
        den = jnp.einsum("bhqf,bhf->bhq", phi_q, z)[..., None] + 1e-6
        o = num / den
        return (lambda x, *d: x.transpose(*d))(o, 0, 2, 1, 3).reshape(B, S, D) @ wo

    def _B_ref(x, w_gate, w_up, w_down):
        return (_gelu(x @ w_gate) * (x @ w_up)) @ w_down

    x = A_x
    h = x + _A_ref(_layernorm(x, axis=-1), A_wqkv, A_w_phi, A_wo)
    h2 = h + _B_ref(_layernorm(h, axis=-1), B_w_gate, B_w_up, B_w_down)
    return h2
```

```python
import functools
import jax
import jax.numpy as jnp
from jax import lax
import jax.experimental.pallas as pl
import jax.experimental.pallas.tpu as pltpu

H = 32
DH = 20
NG = 16
GR = 2 * DH
F32 = jnp.float32
BF16 = jnp.bfloat16

_NT = (((1,), (1,)), ((), ()))


def _ln(x):
    m = jnp.mean(x, axis=-1, keepdims=True)
    xc = x - m
    v = jnp.mean(xc * xc, axis=-1, keepdims=True)
    return xc * lax.rsqrt(v + 1e-5)


def _gelu(x):
    c = 0.7978845608028654
    return 0.5 * x * (1.0 + jnp.tanh(c * (x + 0.044715 * (x * x * x))))


def _recip(x):
    r = pl.reciprocal(x, approx=True)
    return r * (2.0 - x * r)


def _feature_map(p):
    s = [p[8 * j:8 * j + 8] for j in range(5)]

    def red(vals, op):
        a = op(op(vals[0], vals[1]), op(vals[2], vals[3]))
        a = op(a, vals[4])
        a = op(a, pltpu.roll(a, 2, 0))
        a = op(a, pltpu.roll(a, 4, 0))
        return a

    mx = red(s, jnp.maximum)
    mn = red(s, jnp.minimum)
    ep = [jnp.exp(a - mx) for a in s]
    en = [jnp.exp(mn - a) for a in s]
    rp = _recip(red(ep, jnp.add))
    rn = _recip(red(en, jnp.add))
    return jnp.concatenate([a * rp for a in ep] + [a * rn for a in en], axis=0).astype(BF16)


def _kernel(x_hbm, wphi_hbm, wqkv_hbm, wo_hbm, wg_hbm, wu_hbm, wd_hbm,
            out_hbm,
            x_v, wphi_v, wqkv_v, wo_v, wg_v, wu_v, wd_v, out_v, wsems, xsems, osems, fence,
            blk_scr, wall_scr, phiq_scr, kv_scr, a_scr, xn_scr, vt_scr, h_scr, hn_scr,
            *, TS, T2, FC, QSPLIT, ORDER, RELOAD, RA, RB, XP, VS):
    S, D = x_v.shape
    F = wg_v.shape[-1]
    n1 = S // TS
    n2 = S // T2
    TQ = min(TS, T2)

    def qkv_copy(j):
        return pltpu.make_async_copy(wqkv_hbm.at[:, pl.ds(j * D, D)], wqkv_v.at[j], wsems.at[j])

    def x_copy(t):
        return pltpu.make_async_copy(x_hbm.at[0, pl.ds(t * TS, TS), :], x_v.at[pl.ds(t * TS, TS), :], xsems.at[t])

    def out_copy(t):
        return pltpu.make_async_copy(out_v.at[pl.ds(t * T2, T2), :], out_hbm.at[0, pl.ds(t * T2, T2), :], osems.at[t])

    wphi_copy = pltpu.make_async_copy(wphi_hbm, wphi_v, wsems.at[7])
    late = [pltpu.make_async_copy(wo_hbm, wo_v, wsems.at[3]),
            pltpu.make_async_copy(wg_hbm, wg_v, wsems.at[4]),
            pltpu.make_async_copy(wu_hbm, wu_v, wsems.at[5]),
            pltpu.make_async_copy(wd_hbm, wd_v, wsems.at[6])]

    x0a = pltpu.make_async_copy(x_hbm.at[0, pl.ds(0, RA), :], x_v.at[pl.ds(0, RA), :], wsems.at[8])
    x0b = pltpu.make_async_copy(x_hbm.at[0, pl.ds(RA, TS - RA), :], x_v.at[pl.ds(RA, TS - RA), :], xsems.at[0])
    for cp in [x0a, wphi_copy, qkv_copy(2), x0b, qkv_copy(0), qkv_copy(1)] + [x_copy(t) for t in range(1, n1)] + late:
        cp.start()
        pl.semaphore_signal(fence, 1)
        pl.semaphore_wait(fence, 1)
    kv_scr[...] = jnp.zeros_like(kv_scr)

    r = lax.broadcasted_iota(jnp.int32, (160, DH), 0)
    c = lax.broadcasted_iota(jnp.int32, (160, DH), 1)
    rg = (r >= 40).astype(jnp.int32) + (r >= 80).astype(jnp.int32) + (r >= 120).astype(jnp.int32)
    et = jnp.where(((r - 40 * rg) >> 1) == c, 1.0, 0.0).astype(BF16)
    r = lax.broadcasted_iota(jnp.int32, (160, 128), 0)
    c = lax.broadcasted_iota(jnp.int32, (160, 128), 1)
    rg = (r >= 40).astype(jnp.int32) + (r >= 80).astype(jnp.int32) + (r >= 120).astype(jnp.int32)
    lo0 = rg * 40 + (r & 1) * DH
    kk = lax.broadcasted_iota(jnp.int32, (D, D), 0)
    cc = lax.broadcasted_iota(jnp.int32, (D, D), 1)
    perm = jnp.where(cc == (kk & (H - 1)) * DH + (kk >> 5), 1.0, 0.0).astype(BF16)

    def ln_rows(r0, r1):
        xn_scr[r0:r1, :] = _ln(x_v[r0:r1, :].astype(F32)).astype(BF16)

    def v_rows(r0, r1):
        vt_scr[:, r0:r1] = jnp.dot(xn_scr[r0:r1, :], wqkv_v[2], preferred_element_type=F32).T.astype(BF16)

    x0a.wait()
    ln_rows(0, RA)
    wphi_copy.wait()
    w3 = wphi_v[...].astype(F32)
    wr = jnp.concatenate([w3[d] for d in range(DH)], axis=1).astype(BF16)
    xf = jnp.dot(wr, perm, preferred_element_type=F32).astype(BF16)
    for t in range(5):
        full = jnp.dot(et, xf[:, 128 * t:128 * t + 128], preferred_element_type=F32)
        lo = lo0 - 8 * t
        blk_scr[t] = jnp.where((c >= lo) & (c < lo + DH), full, 0.0).astype(BF16)

    def fold(j):
        acc = []
        prev = None
        for t in range(5):
            res = lax.dot_general(blk_scr[t], wqkv_v[j, :, 128 * t:128 * t + 128], _NT,
                                  preferred_element_type=F32)
            acc.append(res[0:40] if prev is None else res[0:40] + prev)
            if t < 4:
                acc.append(res[40:120])
                prev = res[120:160]
            else:
                acc.append(res[40:160])
        wall_scr[j] = jnp.concatenate(acc, axis=0).astype(BF16)

    qkv_copy(2).wait()
    v_rows(0, RA)
    if XP == 0:
        wall_scr[2] = wqkv_v[2].T
    x0b.wait()
    for r0 in range(RA, TS, 128):
        ln_rows(r0, r0 + 128)
    if XP == 1:
        wall_scr[2] = wqkv_v[2].T
    for r0 in range(RA, RB, VS):
        v_rows(r0, r0 + VS)
    qkv_copy(0).wait()
    qkv_copy(1).wait()
    if XP == 2:
        wall_scr[2] = wqkv_v[2].T
    if RB < TS:
        v_rows(RB, TS)
    fold(1)
    fold(0)

    def store_phiq(t, g, ph):
        for u in range(TS // TQ):
            phiq_scr[t * (TS // TQ) + u, g * 2 * GR:(g + 1) * 2 * GR, :] = ph[:, u * TQ:(u + 1) * TQ]

    def kv_update(phik):
        ones = jnp.ones((8, TS), BF16)
        for g in range(NG):
            vt = jnp.concatenate([vt_scr[g * GR:(g + 1) * GR, :], ones], axis=0)
            kv_scr[g] += lax.dot_general(vt, phik[g], _NT, preferred_element_type=F32)

    def p1_body(t, carry):
        x_copy(t + 1).wait()

        xn = xn_scr[...]
        if ORDER == 0:
            xn2 = _ln(x_v[pl.ds(pl.multiple_of((t + 1) * TS, TS), TS), :].astype(F32)).astype(BF16)
            xn_scr[...] = xn2
        pk = lax.dot_general(wall_scr[1], xn, _NT, preferred_element_type=F32)
        if ORDER == 1:
            xn2 = _ln(x_v[pl.ds(pl.multiple_of((t + 1) * TS, TS), TS), :].astype(F32)).astype(BF16)
            xn_scr[...] = xn2
        pq = lax.dot_general(wall_scr[0], xn, _NT, preferred_element_type=F32)
        phik = [_feature_map(pk[g * GR:(g + 1) * GR]) for g in range(NG)]
        kv_update(phik)
        if RELOAD:
            xn2 = xn_scr[...]
        pv = lax.dot_general(wall_scr[2], xn2, _NT, preferred_element_type=F32)
        for g in range(NG):
            store_phiq(t, g, _feature_map(pq[g * GR:(g + 1) * GR]))
        vt_scr[...] = pv.astype(BF16)
        return carry

    lax.fori_loop(0, n1 - 1, p1_body, 0)

    ns = T2 // TQ

    def prep1(t):
        res = []
        for jj in range(ns):
            for g in range(NG):
                ph = phiq_scr[t * ns + jj, g * 2 * GR:(g + 1) * 2 * GR, :]
                res.append(jnp.dot(a_scr[g], ph, preferred_element_type=F32))
        return res

    def prep2(res):
        sub = lax.broadcasted_iota(jnp.int32, (8, TQ), 0) < 4
        os_ = []
        for jj in range(ns):
            pieces = []
            for g in range(NG):
                oe = res[jj * NG + g]
                r = _recip(oe[40:48] + 1e-6)
                rr = pltpu.roll(r, 4, 0)
                ra = jnp.where(sub, r, rr)
                rb = jnp.where(sub, rr, r)
                pieces += [oe[0:8] * ra, oe[8:16] * ra, oe[16:24] * r, oe[24:32] * rb, oe[32:40] * rb]
            ot = jnp.concatenate(pieces, axis=0)
            os_.append(ot.T.astype(BF16))
        o = os_[0] if len(os_) == 1 else jnp.concatenate(os_, axis=0)
        return jnp.dot(o, wo_v[...], preferred_element_type=F32)

    def prep3(t, attn):
        h = x_v[pl.ds(pl.multiple_of(t * T2, T2), T2), :].astype(F32) + attn
        h_scr[...] = h
        hn_scr[...] = _ln(h).astype(BF16)

    for cp in late:
        cp.wait()
    tl = n1 - 1
    xn = xn_scr[...]

    def qpart(g0, g1):
        pq = lax.dot_general(wall_scr[0, g0 * GR:g1 * GR, :], xn, _NT, preferred_element_type=F32)
        for g in range(g0, g1):
            store_phiq(tl, g, _feature_map(pq[(g - g0) * GR:(g - g0 + 1) * GR]))

    pk = lax.dot_general(wall_scr[1], xn, _NT, preferred_element_type=F32)
    phik = [_feature_map(pk[g * GR:(g + 1) * GR]) for g in range(NG)]
    qpart(0, QSPLIT[0])
    kv_update(phik)
    r = lax.broadcasted_iota(jnp.int32, (48, 2 * GR), 0)
    c = lax.broadcasted_iota(jnp.int32, (48, 2 * GR), 1)
    hr = jnp.where(r < 40, (r >= DH).astype(jnp.int32), (r >= 44).astype(jnp.int32))
    mask = hr == (c & 1)
    for g in range(NG):
        a_scr[g] = jnp.where(mask, kv_scr[g], 0.0).astype(BF16)
    res = prep1(0)
    qpart(QSPLIT[0], QSPLIT[1])
    attn = prep2(res)
    qpart(QSPLIT[1], NG)
    prep3(0, attn)

    def ffn_chunk(hn, c):
        g = jnp.dot(hn, wg_v[:, c * FC:(c + 1) * FC], preferred_element_type=F32)
        u = jnp.dot(hn, wu_v[:, c * FC:(c + 1) * FC], preferred_element_type=F32)
        a = (_gelu(g) * u).astype(BF16)
        return jnp.dot(a, wd_v[c * FC:(c + 1) * FC, :], preferred_element_type=F32)

    nc = F // FC

    def p2_body(t, with_prep):
        hn = hn_scr[...]
        if with_prep:
            res = prep1(t + 1)
        acc = h_scr[...] + ffn_chunk(hn, 0)
        if with_prep:
            attn = prep2(res)
        for c in range(1, nc):
            if with_prep and c == nc - 1:
                prep3(t + 1, attn)
            acc = acc + ffn_chunk(hn, c)
        out_v[pl.ds(pl.multiple_of(t * T2, T2), T2), :] = acc.astype(out_v.dtype)
        out_copy(t).start()

    def p2_loop(t, carry):
        p2_body(t, True)
        return carry

    lax.fori_loop(0, n2 - 1, p2_loop, 0)
    p2_body(n2 - 1, False)
    for t in range(n2):
        out_copy(t).wait()


def _impl(A_x, A_wqkv, A_w_phi, A_wo, B_x, B_w_gate, B_w_up, B_w_down, TS=512, T2=256, FC=512, QSPLIT=(2, 6), ORDER=0, RELOAD=False, RA=128, RB=512, XP=2, VS=128):
    B, S, D = A_x.shape
    F = B_w_gate.shape[-1]
    TQ = min(TS, T2)
    anyspec = pl.BlockSpec(memory_space=pl.ANY)
    return pl.pallas_call(
        functools.partial(_kernel, TS=TS, T2=T2, FC=FC, QSPLIT=QSPLIT, ORDER=ORDER, RELOAD=RELOAD, RA=RA, RB=RB, XP=XP, VS=VS),
        in_specs=[anyspec] * 7,
        out_specs=anyspec,
        out_shape=jax.ShapeDtypeStruct((B, S, D), A_x.dtype),
        scratch_shapes=[
            pltpu.VMEM((S, D), BF16),
            pltpu.VMEM((DH, DH, H), BF16),
            pltpu.VMEM((3, D, D), BF16),
            pltpu.VMEM((D, D), BF16),
            pltpu.VMEM((D, F), BF16),
            pltpu.VMEM((D, F), BF16),
            pltpu.VMEM((F, D), BF16),
            pltpu.VMEM((S, D), BF16),
            pltpu.SemaphoreType.DMA((9,)),
            pltpu.SemaphoreType.DMA((S // TS,)),
            pltpu.SemaphoreType.DMA((S // T2,)),
            pltpu.SemaphoreType.REGULAR,
            pltpu.VMEM((5, 160, 128), BF16),
            pltpu.VMEM((3, D, D), BF16),
            pltpu.VMEM((S // TQ, 2 * D, TQ), BF16),
            pltpu.VMEM((NG, 48, 2 * GR), F32),
            pltpu.VMEM((NG, 48, 2 * GR), BF16),
            pltpu.VMEM((TS, D), BF16),
            pltpu.VMEM((D, TS), BF16),
            pltpu.VMEM((T2, D), F32),
            pltpu.VMEM((T2, D), BF16),
        ],
        compiler_params=pltpu.CompilerParams(
            vmem_limit_bytes=100 * 1024 * 1024,
        ),
    )(A_x, jnp.transpose(A_w_phi, (1, 2, 0)), A_wqkv, A_wo, B_w_gate, B_w_up, B_w_down)


@jax.jit
def pallas_sequential_preLN__linear_kernel_hedgehog__geglu_ffn__prompt_kernel(
        A_x, A_wqkv, A_w_phi, A_wo, B_x, B_w_gate, B_w_up, B_w_down):
    return _impl(A_x, A_wqkv, A_w_phi, A_wo, B_x, B_w_gate, B_w_up, B_w_down)
```

```python
import functools
import jax
import jax.numpy as jnp
from jax import lax
import jax.experimental.pallas as pl
import jax.experimental.pallas.tpu as pltpu

H = 32
DH = 20
NG = 16
GR = 2 * DH
KH = 256
F32 = jnp.float32
BF16 = jnp.bfloat16
U32 = jnp.uint32
LOG2E = 1.4426950408889634

_NT = (((1,), (1,)), ((), ()))

_GUESTS = {3: (0, 1, 2), 6: (4, 5, 7), 9: (8, 10, 11), 12: (13, 14, 15)}
_ORDER = ["g0", "g1", "g2", "s0", "s1", "s2", "g3", "g4", "g5", "s4", "s5", "g6", "s7", "g7",
          "g8", "s8", "g9", "s10", "s11", "g10", "g11", "g12", "s13", "s14", "s15", "g13", "g14", "g15"]
_OFF = {}
_o = 0
for _n in _ORDER:
    _OFF[_n] = _o
    _o += 32 if _n[0] == "g" else 8
PR = _o
_HOST = {h: (gg, i) for gg, hs in _GUESTS.items() for i, h in enumerate(hs)}
_RANGES = [(0, 152), (96, 272), (216, 392), (336, 512), (456, 608)]


def _row_tables(width):
    sub = lax.broadcasted_iota(jnp.int32, (8, width), 0)
    pair = sub >> 1
    hl = sub & 1
    fs, hs = [], []
    for n in _ORDER:
        g = int(n[1:])
        if n[0] == "g":
            for j in range(1, 5):
                fs.append(pair + 4 * j)
                hs.append(hl + 2 * g)
        else:
            gg, i = _HOST[g]
            p = 3 - i
            fs.append(jnp.where(pair == p, 1 + i, pair + 1 - (pair > p).astype(jnp.int32)))
            hs.append(jnp.where(pair == p, 2 * gg, 2 * g) + hl)
    return jnp.concatenate(fs, axis=0), jnp.concatenate(hs, axis=0)


def _group_slabs(pt, g):
    pair = lax.broadcasted_iota(jnp.int32, (8, pt.shape[1]), 0) >> 1
    slab = lambda o: pt[o:o + 8]
    if g in _GUESTS:
        a, b, c = [slab(_OFF["s%d" % h]) for h in _GUESTS[g]]
        s0 = jnp.where(pair == 3, a, jnp.where(pair == 2, b, jnp.where(pair == 1, c, 0.0)))
    else:
        s0 = jnp.where(pair == 3 - _HOST[g][1], 0.0, slab(_OFF["s%d" % g]))
    o = _OFF["g%d" % g]
    return [s0] + [slab(o + 8 * j) for j in range(4)]


def _ln(x):
    m = jnp.mean(x, axis=-1, keepdims=True)
    xc = x - m
    v = jnp.mean(xc * xc, axis=-1, keepdims=True)
    return xc * lax.rsqrt(v + 1e-5)


def _ln1(x):
    inv = 1.0 / x.shape[-1]
    m = jnp.sum(x, axis=-1, keepdims=True) * inv
    v = jnp.maximum(jnp.sum(x * x, axis=-1, keepdims=True) * inv - m * m, 0.0)
    return (x - m) * lax.rsqrt(v + 1e-5)


def _gelu(x):
    c = 0.7978845608028654
    return 0.5 * x * (1.0 + jnp.tanh(c * (x + 0.044715 * (x * x * x))))


def _lhs7(a11, a12, a21, a22):
    return [t.astype(BF16) for t in
            (a11 + a22, a21 + a22, a11, a22, a11 + a12, a21 - a11, a12 - a22)]


def _rhs7(b11, b12, b21, b22):
    return [t.astype(BF16) for t in
            (b11 + b22, b11, b12 - b22, b21 - b11, b22, b11 + b12, b21 + b22)]


def _quads(a):
    m, k = a.shape[0] // 2, a.shape[1] // 2
    return a[0:m, 0:k], a[0:m, k:], a[m:, 0:k], a[m:, k:]


def _lsum(a11, a12, a21, a22):
    return [a11 + a22, a21 + a22, a11, a22, a11 + a12, a21 - a11, a12 - a22]


def _rsum(b11, b12, b21, b22):
    return [b11 + b22, b11, b12 - b22, b21 - b11, b22, b11 + b12, b21 + b22]


def _lhs49(a11, a12, a21, a22):
    return [[t.astype(BF16) for t in _lsum(*_quads(s1))] for s1 in _lsum(a11, a12, a21, a22)]


def _comb(m, order=None):
    if order is not None:
        done = {i: m(i) for i in order}
        m = lambda i: done[i]
    m4, m2 = m(4), m(2)
    c21 = m2 + m4
    m5, m3 = m(5), m(3)
    c12 = m3 + m5
    m1 = m(1)
    c11 = (m4 - m5) + (m1 + m(7))
    c22 = (m3 - m2) + (m1 + m(6))
    return jnp.concatenate([jnp.concatenate([c11, c12], axis=1), jnp.concatenate([c21, c22], axis=1)], axis=0)


_SUMMED = (0, 2, 3, 5, 6)


def _dot(a, b):
    return jnp.dot(a, b, preferred_element_type=F32)


def _dot_nt(a, b):
    return lax.dot_general(a, b, _NT, preferred_element_type=F32)


def _recip(x):
    return pl.reciprocal(x, approx=True)


def _pk(x):
    return pltpu.bitcast(x, U32)


def _upk(x):
    return pltpu.bitcast(x, BF16)


def _feature_map(s, query):
    def red(vals, op):
        a = op(op(vals[0], vals[1]), op(vals[2], vals[3]))
        a = op(a, vals[4])
        a = op(a, pltpu.roll(a, 2, 0))
        a = op(a, pltpu.roll(a, 4, 0))
        return a

    mx = red(s, jnp.maximum)
    mn = red(s, jnp.minimum)
    ep = [jnp.exp2(a - mx) for a in s]
    en = [jnp.exp2(mn - a) for a in s]
    sp = red(ep, jnp.add)
    rn = _recip(red(en, jnp.add))
    if query:
        rn = rn * sp
    else:
        rp = _recip(sp)
        ep = [a * rp for a in ep]
    return jnp.concatenate(ep + [a * rn for a in en], axis=0).astype(BF16)


def _kernel(x_hbm, wphi_hbm, wqkv_hbm, wo_hbm, wg_hbm, wu_hbm, wd_hbm,
            out_hbm,
            x_v, wphi_v, wqkv_v, wo_v, wblk_v, wgu3_v, wd3_v, out_v, wsems, xsems, osems, fence,
            blk_scr, sqk_scr, wqk3_scr, sv_scr, wv3_scr, phiq_scr, kv_scr, a_scr,
            xa_scr, xt_scr, x3_scr, vt_scr, h_scr, hq_scr, f32_scr, sa_scr, sd_scr, a3_scr, tw_scr, to_scr, flag_scr,
            *, TS, T2, FC, SC, PB, XP, QB, SCRIPT, RELOAD, WP, RL2, P2S, WOS, TSCRIPT, WQ, WK, WV, NP, LB, LN2, LORD, LSPLIT, SORD, LB2, XSCR):
    S, D = x_v.shape
    F = wd3_v.shape[0]
    n1 = S // TS
    n2 = S // T2
    PH = TS // 2
    HR = T2 // 2
    RA = 128
    K2 = 2 * KH

    def qkv_copy(j):
        return pltpu.make_async_copy(wqkv_hbm.at[:, pl.ds(j * D, D)], wqkv_v.at[j], wsems.at[j])

    def x_copy(t):
        return pltpu.make_async_copy(x_hbm.at[0, pl.ds(t * TS, TS), :], x_v.at[pl.ds(t * TS, TS), :], xsems.at[t])

    def out_copy(t):
        return pltpu.make_async_copy(out_v.at[pl.ds(t * T2, T2), :], out_hbm.at[0, pl.ds(t * T2, T2), :], osems.at[t])

    wphi_copy = pltpu.make_async_copy(wphi_hbm, wphi_v, wsems.at[7])
    late = [pltpu.make_async_copy(wo_hbm, wo_v, wsems.at[3]),
            pltpu.make_async_copy(wg_hbm.at[pl.ds(K2, D - K2), :], wgu3_v.at[0], wsems.at[3]),
            pltpu.make_async_copy(wu_hbm.at[pl.ds(K2, D - K2), :], wgu3_v.at[1], wsems.at[3]),
            pltpu.make_async_copy(wd_hbm.at[:, pl.ds(K2, D - K2)], wd3_v, wsems.at[3])]

    def part_copies(parts, sem):
        cps = []
        for p in parts:
            for u in range(2):
                if p < 6:
                    src = (wg_hbm, wu_hbm)[u].at[pl.ds(0, K2), pl.ds(p * KH, KH)]
                else:
                    src = wd_hbm.at[pl.ds((p - 6) * FC, FC), pl.ds(u * KH, KH)]
                cps.append(pltpu.make_async_copy(src, wblk_v.at[p, u], sem))
        return cps

    groups = [part_copies((0,), wsems.at[4]), part_copies(range(1, 1 + NP), wsems.at[5]),
              part_copies(range(1 + NP, 1 + 2 * NP), wsems.at[6])]
    late += part_copies(range(1 + 2 * NP, 9), wsems.at[3])
    slot = lambda p: ((p + NP - 1) // NP, (p + NP - 1) % NP)

    step = pl.program_id(0)
    tw_u, sa_u, sd_u, a3_u, phiq_u, wd3_u = [
        r.bitcast(U32) for r in (tw_scr, sa_scr, sd_scr, a3_scr, phiq_scr, wd3_v)]
    sqk_u, wqk3_u, sv_u, wv3_u, xt_u, x3_u, vt_u = [
        r.bitcast(U32) for r in (sqk_scr, wqk3_scr, sv_scr, wv3_scr, xt_scr, x3_scr, vt_scr)]

    def x_operands(x1, x2):
        return [[t[:, 128 * k:128 * k + 128].astype(BF16) for k in range(2)]
                for t in _rsum(x1[:, 0:KH], x2[:, 0:KH], x1[:, KH:K2], x2[:, KH:K2])]

    @pl.when(step == 0)
    def _prologue():
        x0a = pltpu.make_async_copy(x_hbm.at[0, pl.ds(0, RA), :], x_v.at[pl.ds(0, RA), :], wsems.at[8])
        x0b = pltpu.make_async_copy(x_hbm.at[0, pl.ds(RA, TS - RA), :], x_v.at[pl.ds(RA, TS - RA), :], xsems.at[0])
        for cp in ([x0a, wphi_copy, qkv_copy(2), x0b, qkv_copy(0), qkv_copy(1)]
                   + [cp for t in range(1, n1) for cp in [x_copy(t)] + groups[t - 1]] + late):
            cp.start()
            pl.semaphore_signal(fence, 1)
            pl.semaphore_wait(fence, 1)
        kv_scr[...] = jnp.zeros_like(kv_scr)
        flag_scr[...] = jnp.zeros_like(flag_scr)
        vt_scr[:, :, :, GR:GR + 8, :] = jnp.ones((2, TS // QB, NG, 8, QB), BF16)

        fcol, _ = _row_tables(DH)
        c = lax.broadcasted_iota(jnp.int32, (PR, DH), 1)
        et = jnp.where(c == fcol, 1.0, jnp.where(c == 0, -1.0, 0.0))
        _, hcol = _row_tables(128)
        lo0 = hcol * DH
        kk = lax.broadcasted_iota(jnp.int32, (D, D), 0)
        cc = lax.broadcasted_iota(jnp.int32, (D, D), 1)
        perm = jnp.where(cc == (kk & (H - 1)) * DH + (kk >> 5), 1.0, 0.0).astype(BF16)

        def v_rows(xn, r0):
            vt = _dot(xn.astype(BF16), wqkv_v[2]).T.astype(BF16)
            for g in range(NG):
                vt_scr[0, r0 // RA, g, 0:GR, :] = vt[g * GR:(g + 1) * GR]

        def v_weights():
            wvt = wqkv_v[2].T
            hv = D // 2
            for r0 in range(0, hv, 32):
                q = [wvt[h0 + r0:h0 + r0 + 32, k0:k0 + KH].astype(F32) for h0 in (0, hv) for k0 in (0, KH)]
                for i, sv in enumerate(_lsum(*q)):
                    for k in range(2):
                        sv_scr[i, k, r0:r0 + 32, :] = sv[:, 128 * k:128 * k + 128].astype(BF16)
            wv3_scr[...] = wvt[:, K2:]

        x0a.wait()
        xa_scr[...] = _ln1(x_v[0:RA, :].astype(F32))
        wphi_copy.wait()
        w3 = wphi_v[...].astype(F32)
        wr = jnp.concatenate([w3[d] for d in range(DH)], axis=1).astype(BF16)
        xf = _dot(wr, perm).astype(BF16)
        for t, (r0, r1) in enumerate(_RANGES):
            full = _dot(et[r0:r1].astype(BF16), xf[:, 128 * t:128 * t + 128])
            lo = lo0[r0:r1] - 128 * t
            c = lax.broadcasted_iota(jnp.int32, (r1 - r0, 128), 1)
            blk_scr[t, 0:r1 - r0, :] = jnp.where((c >= lo) & (c < lo + DH), full * LOG2E, 0.0).astype(BF16)

        qkv_copy(2).wait()
        v_rows(xa_scr[...], 0)
        if XP == 0:
            v_weights()
        x0b.wait()
        xs = [xa_scr[...]] + [_ln1(x_v[r0:r0 + RA, :].astype(F32)) for r0 in range(RA, TS, RA)]
        if XP == 1:
            v_weights()
        for j in range(1, TS // RA):
            v_rows(xs[j], j * RA)
        for j in range(PH // RA):
            for i, tv in enumerate(x_operands(xs[j], xs[j + PH // RA])):
                for k in range(2):
                    xt_scr[0, i, k, j * RA:(j + 1) * RA, :] = tv[k]
        for j in range(TS // RA):
            x3_scr[0, j * RA:(j + 1) * RA, :] = xs[j][:, K2:].astype(BF16)
        qkv_copy(0).wait()
        qkv_copy(1).wait()
        if XP == 2:
            v_weights()
        prev = None
        done = 0
        for t, (r0, r1) in enumerate(_RANGES):
            res = [_dot_nt(blk_scr[t, 0:r1 - r0, :], wqkv_v[j, :, 128 * t:128 * t + 128]) for j in range(2)]
            if prev is not None:
                a, b = r0 - done, prev[0].shape[0] - (r0 - done)
                res = [jnp.concatenate(([prev[j][0:a]] if a else []) + [res[j][0:b] + prev[j][a:], res[j][b:]], axis=0)
                       for j in range(2)]
            end = _RANGES[t + 1][0] // 16 * 16 if t < 4 else r1
            wq, wk = [res[j][0:end - done] for j in range(2)]
            prev = [res[j][end - done:] for j in range(2)] if t < 4 else None
            for i, sv in enumerate(_lsum(wq[:, 0:KH], wq[:, KH:K2], wk[:, 0:KH], wk[:, KH:K2])):
                for k in range(2):
                    sqk_scr[i, k, done:end, :] = sv[:, 128 * k:128 * k + 128].astype(BF16)
            for j, w in enumerate((wq, wk)):
                wqk3_scr[j, done:end, :] = w[:, K2:].astype(BF16)
            done = end

    def fmaps(pt, query=False):
        return [_feature_map(_group_slabs(pt, g), query) for g in range(NG)]

    def store_phiq(idx, c0, pt):
        for g, ph in enumerate(fmaps(pt, True)):
            phiq_scr[idx * nb + c0 // QB, g * 2 * GR:(g + 1) * 2 * GR, :] = ph

    def kv_update(phik, cur, which=None):
        for g in range(NG):
            acc = kv_scr[g]
            for j, p in enumerate(phik):
                if which is not None and j not in which:
                    continue
                acc = acc + _dot_nt(_upk(vt_u[cur, j, g]), p[g])
            kv_scr[g] = acc

    def store_vt(nxt, g0, c0, v):
        for g in range(NG // 2):
            vt_scr[nxt, c0 // QB, g0 + g, 0:GR, :] = v[g * GR:(g + 1) * GR].astype(BF16)

    nb = PH // QB
    qh = QB // 2

    def qk_ops(j, cur):
        m = lambda i: sum(_dot_nt(_upk(sqk_u[i - 1, k]), _upk(xt_u[cur, i - 1, k, j * qh:(j + 1) * qh, :]))
                          for k in range(2))
        r = lambda w, half: _dot_nt(_upk(wqk3_u[w]),
                                    _upk(x3_u[cur, half * PH // 2 + j * qh:half * PH // 2 + (j + 1) * qh, :]))
        return m, r

    fh = FC // 2

    _RS = ((0, 3, 1), (0, None, 1), (1, 3, -1), (2, 0, -1), (3, None, 1), (0, 1, 1), (2, 3, 1))

    def weight_prep(parts, ys):
        blocks = []
        for p in parts:
            if p is None:
                blocks += [(p, r0, 0) for r0 in range(0, KH, PB)]
            else:
                blocks += [(p, r0, i) for i in range(7) for r0 in range(0, 128, PB)]
        for bi, (part, r0, i) in enumerate(blocks):
            y = ys[bi * len(ys) // len(blocks)]
            z = pltpu.bitcast(pltpu.bitcast(y, U32) & flag_scr[...], F32)
            z = jnp.concatenate([z] * (PB // 8), axis=0)
            if part is None:
                q = [wo_v[k0 + r0:k0 + r0 + PB, n0:n0 + KH].astype(F32) for k0 in (0, KH) for n0 in (0, KH)]
                z = jnp.concatenate([z, z], axis=1)
                q[0] = q[0] + z
                q[3] = q[3] + z
                tv = _rhs7(*q)
                for k, p in enumerate(_SUMMED):
                    to_scr[k, r0:r0 + PB, :] = tv[p]
                continue

            def src(qi):
                k0 = (qi // 2) * KH + r0
                return jnp.concatenate(
                    [wblk_v[part[0], qi % 2, k0 + d:k0 + d + PB, :].astype(F32) for d in (0, 128)], axis=0)

            qa, qb, sg = _RS[i]
            s1 = src(qa) if qb is None else (src(qa) + src(qb) if sg > 0 else src(qa) - src(qb))
            b11, b12, b21, b22 = _quads(s1)
            for j, s2 in enumerate(_rsum(b11 + z, b12, b21, b22 + z)):
                tw_scr[part[1], part[2], 7 * i + j, r0:r0 + PB, :] = s2.astype(BF16)

    def pick(a, ncols, per):
        nr = a.shape[0] // 8
        return [a[8 * (i * nr // per):8 * (i * nr // per) + 8, 128 * j:128 * j + 128]
                for j in range(ncols) for i in range(per)]

    def qk_token(tok, t, cur, M, phik):
        j = "ab".index(tok[0])
        m, r = qk_ops(j, cur)
        what = tok[1:]
        if what == "k1":
            phik[j] = fmaps(M[j, 2] + M[j, 4] + r(1, 0))
        elif what == "q2":
            store_phiq(2 * t + 1, j * QB, M[j, 3] + M[j, 5] + r(0, 1))
        elif what == "q1":
            store_phiq(2 * t, j * QB, (M[j, 4] - M[j, 5] + M[j, 1]) + M[j, 7] + r(0, 0))
        elif what == "k2":
            phik[nb + j] = fmaps((M[j, 3] - M[j, 2] + M[j, 1]) + M[j, 6] + r(1, 1))
        else:
            M[j, int(what)] = m(int(what))

    @pl.when(jnp.logical_and(step >= 1, step < n1))
    def _p1():
        t = step - 1
        cur = t % 2
        nxt = 1 - cur
        hv = D // 2
        x_copy(t + 1).wait()
        for k in range(n1 - 1):
            @pl.when(t == k)
            def _():
                for cp in groups[k]:
                    cp.wait()

        phik = [None] * (2 * nb)
        M = {}
        V = {}
        for tok in SCRIPT.split():
            if tok[:2] == "kv":
                kv_update(phik, cur, [int(c) for c in tok[2:]] or None)
            elif tok[0] == "V":
                j = "ab".index(tok[1])
                base = pl.multiple_of((t + 1) * TS, TS)
                xn = [_ln1(x_v[pl.ds(base + h0 + j * QB, QB), :].astype(F32)) for h0 in (0, PH)]
                if XSCR:
                    for hh in range(2):
                        f32_scr[j, hh * QB:(hh + 1) * QB, :] = xn[hh][:, 0:K2]
                    xt = x_operands(f32_scr[j, 0:QB, :], f32_scr[j, QB:, :])
                else:
                    xt = x_operands(xn[0], xn[1])
                x3 = [xn[hh][:, K2:].astype(BF16) for hh in range(2)]
                for i in range(7):
                    for k in range(2):
                        xt_scr[nxt, i, k, j * QB:(j + 1) * QB, :] = xt[i][k]
                for hh in range(2):
                    x3_scr[nxt, hh * PH + j * QB:hh * PH + (j + 1) * QB, :] = x3[hh]
                if RELOAD:
                    xk = lambda i, k: _upk(xt_u[nxt, i, k, j * qh:(j + 1) * qh, :])
                    x3 = [_upk(x3_u[nxt, hh * PH // 2 + j * qh:hh * PH // 2 + (j + 1) * qh, :]) for hh in range(2)]
                else:
                    xk = lambda i, k: xt[i][k]
                v = lambda i: sum(_dot_nt(_upk(sv_u[i - 1, k]), xk(i - 1, k)) for k in range(2))
                v2 = v(2)
                v4 = v(4)
                r1 = _dot_nt(_upk(wv3_u[...]), x3[0])
                store_vt(nxt, NG // 2, j * QB, v2 + v4 + r1[hv:])
                v5 = v(5)
                v3 = v(3)
                r2 = _dot_nt(_upk(wv3_u[...]), x3[1])
                store_vt(nxt, 0, PH + j * QB, v3 + v5 + r2[0:hv])
                v1 = v(1)
                V[j] = [v2, v4, r1, v5, v3, r2, v1]
                store_vt(nxt, 0, j * QB, (v4 - v5 + r1[0:hv]) + (v1 + v(7)))
                store_vt(nxt, NG // 2, PH + j * QB, (v3 - v2 + r2[hv:]) + (v1 + v(6)))
            else:
                qk_token(tok, t, cur, M, phik)
        ys = (pick(M[0, 4], 1, WQ[0]) + [y for k in WK for y in pick(M[k], 1, WQ[1])]
              + [y for k in WV for y in pick(V[0][k], 1, WQ[2])] + [y for k in WV for y in pick(V[1][k], 1, WQ[3])])
        weight_prep([(jnp.maximum(NP * (t - 1) + 1 + k, 0), t, k) for k in range(NP)], ys)

    def prep1(t):
        return [jnp.concatenate([_dot(a_scr[g], _upk(phiq_u[t * nb + j, g * GR:(g + 1) * GR, :]))
                                 for j in range(nb)], axis=1) for g in range(NG)]

    def normalize(res, sub):
        pieces = []
        for oe in res:
            r = _recip(oe[40:48])
            rr = pltpu.roll(r, 4, 0)
            ra = jnp.where(sub, r, rr)
            rb = jnp.where(sub, rr, r)
            pieces += [oe[0:8] * ra, oe[8:16] * ra, oe[16:24] * r, oe[24:32] * rb, oe[32:40] * rb]
        return jnp.concatenate(pieces, axis=0)

    def prep2(res, tap=None):
        ot = normalize(res, lax.broadcasted_iota(jnp.int32, (8, T2), 0) < 4)
        o = ot.T.astype(BF16)
        if not WOS:
            return _dot(o, wo_v[...])
        a11, a12, a21, a22 = ot[0:KH, 0:HR], ot[KH:K2, 0:HR], ot[0:KH, HR:], ot[KH:K2, HR:]
        tr = lambda a: a.T.astype(BF16)
        r3 = _dot(o, wo_v[:, K2:])
        rk = _dot(o[:, K2:], wo_v[K2:, 0:K2])
        m1 = _dot(tr(a11 + a22), to_scr[0])
        m4 = _dot(o[HR:, KH:K2], to_scr[2])
        m5 = _dot(tr(a11 + a12), wo_v[KH:K2, KH:K2])
        m7 = _dot(tr(a12 - a22), to_scr[4])
        m3 = _dot(o[0:HR, 0:KH], to_scr[1])
        m2 = _dot(tr(a21 + a22), wo_v[0:KH, 0:KH])
        m6 = _dot(tr(a21 - a11), to_scr[3])
        if tap is not None:
            tap += [r3, rk, m1, m4, m5, m7, m3, m2]
        top = jnp.concatenate([m1 + m4 - m5 + m7, m3 + m5], axis=1)
        bot = jnp.concatenate([m2 + m4, m1 - m2 + m3 + m6], axis=1)
        return jnp.concatenate([jnp.concatenate([top, bot], axis=0) + rk, r3], axis=1)

    _LS = ((0, 3, 1), (2, 3, 1), (0, None, 1), (3, None, 1), (0, 1, 1), (2, 0, -1), (1, 3, -1))

    def store49(dst, src):
        q = HR // 2
        for i in SORD:
            for r0 in range(0, q, LB):
                quad = lambda u: jnp.concatenate(
                    [src[(u // 2) * HR + d + r0:(u // 2) * HR + d + r0 + LB, (u % 2) * KH:(u % 2 + 1) * KH]
                     for d in (0, q)], axis=0)
                qa, qb, sg = _LS[i - 1]
                s1 = quad(qa) if qb is None else (quad(qa) + quad(qb) if sg > 0 else quad(qa) - quad(qb))
                for j, s2 in enumerate(_lsum(*_quads(s1))):
                    dst[7 * (i - 1) + j, r0:r0 + LB, :] = s2.astype(BF16)

    def load_sa():
        return [[_upk(sa_u[7 * i + j]) for j in range(7)] for i in range(7)], _upk(a3_u[...])

    def prep3(t, attn):
        hq_scr[...] = x_v[pl.ds(pl.multiple_of(t * T2, T2), T2), :].astype(F32) + attn
        for r0 in range(0, T2, LB2):
            hn = (_ln1 if LN2 & 1 else _ln)(hq_scr[r0:r0 + LB2, :])
            a3_scr[r0:r0 + LB2, :] = hn[:, K2:].astype(BF16)
            f32_scr[3, r0:r0 + LB2, :] = hn[:, 0:K2]
        store49(sa_scr, f32_scr.at[3])
        return (hq_scr[...],) + load_sa()

    nc = F // FC

    def rems(a3, c):
        return {(u, b): _dot(a3, wgu3_v[u, :, b * 256:(b + 1) * 256])
                for b in range(c * FC // 256, (c + 1) * FC // 256) for u in range(2)}

    def rem3(a1, a2, c):
        return _dot(jnp.concatenate([a1, a2], axis=0).astype(BF16), _upk(wd3_u[c * FC // 2:(c + 1) * FC // 2, :]))

    def gate_up(sa, a3, c, tap=None, top_first=False, rem=None):
        a1, a2 = [], []
        for b in range(c * FC // 256, (c + 1) * FC // 256):
            cols = slice(b * 256, (b + 1) * 256)
            m = lambda i: _comb(lambda j: _dot(sa[i - 1][j - 1], _upk(tw_u[slot(b) + (7 * (i - 1) + j - 1,)])))
            if top_first:
                m5 = m(5)
                m3 = m(3)
            m4 = m(4)
            m2 = m(2)
            rg = _dot(a3, wgu3_v[0, :, cols]) if rem is None else rem[0, b]
            g2 = m2 + m4 + rg[HR:]
            if not top_first:
                m5 = m(5)
                m3 = m(3)
            ru = _dot(a3, wgu3_v[1, :, cols]) if rem is None else rem[1, b]
            u1 = m3 + m5 + ru[0:HR]
            m1 = m(1)
            m7 = m(7)
            g1 = (m4 - m5 + rg[0:HR]) + (m1 + m7)
            m6 = m(6)
            u2 = (m3 - m2 + ru[HR:]) + (m1 + m6)
            if tap is not None:
                tap.append([m5, m3, m4, m2, rg, ru, m1, m7, m6])
            a1.append(_gelu(g1) * u1)
            a2.append(_gelu(g2) * u2)
        return jnp.concatenate(a1, axis=1), jnp.concatenate(a2, axis=1)

    def down(acts, tap=None, r3s=None, order=None):
        for a1, a2, c in acts:
            f32_scr[c, 0:HR, :] = a1
            f32_scr[c, HR:, :] = a2
            store49(sd_scr.at[c], f32_scr.at[c])
        sd = [[[_upk(sd_u[c, 7 * i + j]) for j in range(7)] for i in range(7)] for a1, a2, c in acts]
        r3 = sum((r3s or {}).get(a[2]) if a[2] in (r3s or {}) else rem3(*a) for a in acts)

        def m(i):
            v = _comb(lambda j: sum(_dot(sd[k][i - 1][j - 1], _upk(tw_u[slot(6 + acts[k][2]) + (7 * (i - 1) + j - 1,)]))
                                    for k in range(len(acts))), order)
            if tap is not None:
                tap.append(v)
            return v

        return jnp.concatenate([_comb(m, order), r3], axis=1)

    @pl.when(step == n1)
    def _trans():
        for cp in late:
            cp.wait()
        t = n1 - 1
        cur = t % 2
        phik = [None] * (2 * nb)
        M = {}
        st = {}
        sub = lax.broadcasted_iota(jnp.int32, (8, QB), 0) < 4
        tap_g = []
        for tok in TSCRIPT.split():
            if tok[:2] == "kv":
                kv_update(phik, cur, [int(c) for c in tok[2:]] or None)
            elif tok == "mid":
                r = lax.broadcasted_iota(jnp.int32, (48, 2 * GR), 0)
                c = lax.broadcasted_iota(jnp.int32, (48, 2 * GR), 1)
                hr = jnp.where(r < 40, (r >= DH).astype(jnp.int32), (r >= 44).astype(jnp.int32))
                mask = hr == (c & 1)
                eps = jnp.where((r >= 40) & (c < GR), 1e-6, 0.0)
                for g in range(NG):
                    a_scr[g] = jnp.where(mask, kv_scr[g] + eps, 0.0).astype(BF16)
            elif tok[0] == "o":
                j = int(tok[1])
                st[tok] = [_dot(a_scr[g], _upk(phiq_u[j, g * GR:(g + 1) * GR, :])) for g in range(NG)]
            elif tok[0] == "w":
                st[tok] = _dot(normalize(st["o" + tok[1]], sub).T.astype(BF16), wo_v[...])
            elif tok == "ffn":
                h, sa, a3 = prep3(0, jnp.concatenate([st["w%d" % j] for j in range(nb)], axis=0))
                a1, a2 = gate_up(sa, a3, 0, tap_g, True)
                md = []
                h_scr[...] = h + down([(a1, a2, 0)], md)
            else:
                qk_token(tok, t, cur, M, phik)
        ys = (pick(M[0, 4], 1, WP[0]) + [y for k in WK for y in pick(M[k], 1, WP[1])]
              + [y for j in range(nb) for y in pick(st["w%d" % j], 4, WP[2])])
        weight_prep([None] + [(p,) + slot(p) for p in range(1 + 2 * NP, 9)], ys)

    def p2_body(t, with_prep):
        sa, a3 = load_sa()
        if with_prep:
            res = prep1(t + 1)
        if P2S == 0 or not with_prep:
            acts = [gate_up(sa, a3, c) + (c,) for c in range(1, nc)]
            if with_prep:
                attn = prep2(res)
            o = down(acts)
        else:
            acts = [gate_up(sa, a3, 1) + (1,)]
            attn = prep2(res)
            rem = rems(a3, 2)
            r3s = {1: rem3(*acts[0])} if P2S == 1 else None
            acts.append(gate_up(sa, a3, 2, rem=rem) + (2,))
            o = down(acts, r3s=r3s)
        out_v[pl.ds(pl.multiple_of(t * T2, T2), T2), :] = (h_scr[...] + o).astype(out_v.dtype)
        out_copy(t).start()
        if with_prep:
            h, sa, a3 = prep3(t + 1, attn)
            h_scr[...] = h + down([gate_up(sa, a3, 0) + (0,)])

    @pl.when(jnp.logical_and(step > n1, step < n1 + n2))
    def _p2():
        p2_body(step - n1 - 1, True)

    @pl.when(step == n1 + n2)
    def _last():
        sa, a3 = load_sa()
        acts = [gate_up(sa, a3, c) + (c,) for c in range(1, nc)]
        o = h_scr[...] + down(acts, order=LORD)
        base = (n2 - 1) * T2
        tails = []
        for i, (r0, r1, c0, c1) in enumerate(LSPLIT):
            out_v[base + r0:base + r1, c0:c1] = o[r0:r1, c0:c1].astype(out_v.dtype)
            cp = pltpu.make_async_copy(out_v.at[pl.ds(base + r0, r1 - r0), pl.ds(c0, c1 - c0)],
                                       out_hbm.at[0, pl.ds(base + r0, r1 - r0), pl.ds(c0, c1 - c0)],
                                       osems.at[n2 - 1 + i])
            cp.start()
            tails.append(cp)
        for t in range(n2 - 1):
            out_copy(t).wait()
        for cp in tails:
            cp.wait()


_QK = "a4 a2 ak1 a5 a3 aq2 a1 a6 ak2 a7 aq1 b4 b2 bk1 b5 b3 bq2 b1 b6 bk2 b7 bq1 kv021 kv3 "
_SCRIPT = _QK + "Va Vb"
_TSCRIPT = _QK + "mid o0 o1 w0 w1 ffn"


def _impl(A_x, A_wqkv, A_w_phi, A_wo, B_x, B_w_gate, B_w_up, B_w_down, FC=512, SC=256, PB=16, XP=1, QB=128,
          SCRIPT=_SCRIPT, RELOAD=True, WP=(30, 2, 9), RL2=True,
          P2S=0, WOS=True, TSCRIPT=_TSCRIPT,
          WQ=(30, 2, 4, 12),
          WK=((0, 2), (0, 5), (0, 3), (0, 1), (0, 7), (0, 6), (1, 4), (1, 2), (1, 5), (1, 3), (1, 1), (1, 6), (1, 7)),
          WV=(0, 1, 2, 3, 4, 5, 6), NP=3, LB=16, LN2=1,
          SORD=(4, 2, 5, 3, 1, 7, 6), LB2=256, XSCR=True, LORD=(4, 5, 3, 1, 7, 2, 6), LSPLIT=((128, 256, 512, 640), (0, 128, 0, 640), (128, 256, 0, 256),
                                              (128, 192, 256, 512), (192, 256, 256, 512))):
    B, S, D = A_x.shape
    F = B_w_gate.shape[-1]
    TS, T2 = 512, 256
    anyspec = pl.BlockSpec(memory_space=pl.ANY)
    return pl.pallas_call(
        functools.partial(_kernel, TS=TS, T2=T2, FC=FC, SC=SC, PB=PB, XP=XP, QB=QB, SCRIPT=SCRIPT, RELOAD=RELOAD, WP=WP, RL2=RL2, P2S=P2S, WOS=WOS, TSCRIPT=TSCRIPT, WQ=WQ, WK=WK, WV=WV, NP=NP, LB=LB, LN2=LN2, SORD=SORD, LB2=LB2, XSCR=XSCR, LORD=LORD, LSPLIT=LSPLIT),
        grid=(S // TS + S // T2 + 1,),
        in_specs=[anyspec] * 7,
        out_specs=anyspec,
        out_shape=jax.ShapeDtypeStruct((B, S, D), A_x.dtype),
        scratch_shapes=[
            pltpu.VMEM((S, D), BF16),
            pltpu.VMEM((DH, DH, H), BF16),
            pltpu.VMEM((3, D, D), BF16),
            pltpu.VMEM((D, D), BF16),
            pltpu.VMEM((9, 2, 2 * KH, KH), BF16),
            pltpu.VMEM((2, D - 2 * KH, F), BF16),
            pltpu.VMEM((F, D - 2 * KH), BF16),
            pltpu.VMEM((S, D), BF16),
            pltpu.SemaphoreType.DMA((9,)),
            pltpu.SemaphoreType.DMA((S // TS,)),
            pltpu.SemaphoreType.DMA((S // T2 - 1 + len(LSPLIT),)),
            pltpu.SemaphoreType.REGULAR,
            pltpu.VMEM((5, 176, 128), BF16),
            pltpu.VMEM((7, 2, PR, 128), BF16),
            pltpu.VMEM((2, PR, D - 2 * KH), BF16),
            pltpu.VMEM((7, 2, D // 2, 128), BF16),
            pltpu.VMEM((D, D - 2 * KH), BF16),
            pltpu.VMEM((S // QB, 2 * D, QB), BF16),
            pltpu.VMEM((NG, 48, 2 * GR), F32),
            pltpu.VMEM((NG, 48, 2 * GR), BF16),
            pltpu.VMEM((128, D), F32),
            pltpu.VMEM((2, 7, 2, TS // 2, 128), BF16),
            pltpu.VMEM((2, TS, D - 2 * KH), BF16),
            pltpu.VMEM((2, TS // QB, NG, 48, QB), BF16),
            pltpu.VMEM((T2, D), F32),
            pltpu.VMEM((T2, D), F32),
            pltpu.VMEM((4, T2, 2 * KH), F32),
            pltpu.VMEM((49, T2 // 4, 128), BF16),
            pltpu.VMEM((F // FC, 49, T2 // 4, 128), BF16),
            pltpu.VMEM((T2, D - 2 * KH), BF16),
            pltpu.VMEM(((8 + 2 * NP - 1) // NP, NP, 49, 128, 128), BF16),
            pltpu.VMEM((5, KH, KH), BF16),
            pltpu.VMEM((8, 128), U32),
        ],
        compiler_params=pltpu.CompilerParams(
            dimension_semantics=("arbitrary",),
            vmem_limit_bytes=100 * 1024 * 1024,
            disable_bounds_checks=True,
            disable_semaphore_checks=True,
        ),
    )(A_x, jnp.transpose(A_w_phi, (1, 2, 0)), A_wqkv, A_wo, B_w_gate, B_w_up, B_w_down)


@jax.jit
def pallas_sequential_preLN__linear_kernel_hedgehog__geglu_ffn__prompt_kernel(
        A_x, A_wqkv, A_w_phi, A_wo, B_x, B_w_gate, B_w_up, B_w_down):
    return _impl(A_x, A_wqkv, A_w_phi, A_wo, B_x, B_w_gate, B_w_up, B_w_down)
```

```python
import jax
import jax.numpy as jnp
from jax import lax
import jax.experimental.pallas as pl
import jax.experimental.pallas.tpu as pltpu

H = 32
DH = 20
NG = 16
GR = 2 * DH
KH = 256
K2 = 2 * KH
TS = 512
T2 = 256
QB = 128
FC = 512
PB = 16
NP = 3
F32 = jnp.float32
BF16 = jnp.bfloat16
U32 = jnp.uint32
LOG2E = 1.4426950408889634

_NT = (((1,), (1,)), ((), ()))

_GUESTS = {3: (0, 1, 2), 6: (4, 5, 7), 9: (8, 10, 11), 12: (13, 14, 15)}
_ORDER = ["g0", "g1", "g2", "s0", "s1", "s2", "g3", "g4", "g5", "s4", "s5", "g6", "s7", "g7",
          "g8", "s8", "g9", "s10", "s11", "g10", "g11", "g12", "s13", "s14", "s15", "g13", "g14", "g15"]
_OFF = {}
_o = 0
for _n in _ORDER:
    _OFF[_n] = _o
    _o += 32 if _n[0] == "g" else 8
PR = _o
_HOST = {h: (gg, i) for gg, hs in _GUESTS.items() for i, h in enumerate(hs)}
_RANGES = [(0, 152), (96, 272), (216, 392), (336, 512), (456, 608)]

_LS = ((0, 3, 1), (2, 3, 1), (0, None, 1), (3, None, 1), (0, 1, 1), (2, 0, -1), (1, 3, -1))
_RS = ((0, 3, 1), (0, None, 1), (1, 3, -1), (2, 0, -1), (3, None, 1), (0, 1, 1), (2, 3, 1))
_SUMMED = (0, 2, 3, 5, 6)

_KEYS = "a4 a2 a21 a5 a3 a12 a1 a7 a11 a6 a22 b4 b2 b21 b5 b3 b12 b1 b7 b11 b6 b22 "
_SCRIPT1 = "q0 q1 q2 q3 " + _KEYS + "kv021 kv3 Va Vb"
_SCRIPT2 = _KEYS + "q0 q1 q2 q3 kv0123 Mid o0 o1 w0 w1 ffn"
_V_ORDER = "L0 s4 2 4 c21 L1 s3 5 3 c12 s176 1 7 c11 6 c22"
_GU_ORDER = ("4517g3u26", "5342176gu", "4517326gu")
_LAST_ORDER = (4, 5, 3, 1, 7, 2, 6)
_LAST_SPLIT = ((128, 256, 512, 640), (0, 128, 0, 640), (128, 256, 0, 256), (128, 192, 256, 512),
               (192, 256, 256, 512))
_PINS1 = (16, 1, 3, 12, 1)
_PINS2 = (10, 0, 9, 20)


def _row_tables(width):
    sub = lax.broadcasted_iota(jnp.int32, (8, width), 0)
    pair = sub >> 1
    hl = sub & 1
    fs, hs = [], []
    for n in _ORDER:
        g = int(n[1:])
        if n[0] == "g":
            for j in range(1, 5):
                fs.append(pair + 4 * j)
                hs.append(hl + 2 * g)
        else:
            gg, i = _HOST[g]
            p = 3 - i
            fs.append(jnp.where(pair == p, 1 + i, pair + 1 - (pair > p).astype(jnp.int32)))
            hs.append(jnp.where(pair == p, 2 * gg, 2 * g) + hl)
    return jnp.concatenate(fs, axis=0), jnp.concatenate(hs, axis=0)


def _group_slabs(pt, g, base):
    pair = lax.broadcasted_iota(jnp.int32, (8, pt.shape[1]), 0) >> 1
    slab = lambda o: pt[o - base:o - base + 8]
    if g in _GUESTS:
        a, b, c = [slab(_OFF["s%d" % h]) for h in _GUESTS[g]]
        s0 = jnp.where(pair == 3, a, jnp.where(pair == 2, b, jnp.where(pair == 1, c, 0.0)))
    else:
        s0 = jnp.where(pair == 3 - _HOST[g][1], 0.0, slab(_OFF["s%d" % g]))
    o = _OFF["g%d" % g]
    return [s0] + [slab(o + 8 * j) for j in range(4)]


def _ln(x):
    inv = 1.0 / x.shape[-1]
    m = jnp.sum(x, axis=-1, keepdims=True) * inv
    v = jnp.maximum(jnp.sum(x * x, axis=-1, keepdims=True) * inv - m * m, 0.0)
    return (x - m) * lax.rsqrt(v + 1e-5)


def _geglu2(x, u):
    c = 0.7978845608028654
    w = x * u
    return w + w * jnp.tanh(x * (x * x * (c * 0.044715) + c))


def _quads(a):
    m, k = a.shape[0] // 2, a.shape[1] // 2
    return a[0:m, 0:k], a[0:m, k:], a[m:, 0:k], a[m:, k:]


def _lsum(a11, a12, a21, a22):
    return [a11 + a22, a21 + a22, a11, a22, a11 + a12, a21 - a11, a12 - a22]


def _rsum(b11, b12, b21, b22):
    return [b11 + b22, b11, b12 - b22, b21 - b11, b22, b11 + b12, b21 + b22]


def _pair_sum(table, i, quad):
    qa, qb, sg = table[i]
    return quad(qa) if qb is None else (quad(qa) + quad(qb) if sg > 0 else quad(qa) - quad(qb))


def _comb(m, order=None):
    if order is not None:
        done = {i: m(i) for i in order}
        m = lambda i: done[i]
    m4, m2 = m(4), m(2)
    c21 = m2 + m4
    m5, m3 = m(5), m(3)
    c12 = m3 + m5
    m1 = m(1)
    c11 = (m4 - m5) + (m1 + m(7))
    c22 = (m3 - m2) + (m1 + m(6))
    return jnp.concatenate([jnp.concatenate([c11, c12], axis=1), jnp.concatenate([c21, c22], axis=1)], axis=0)


def _dot(a, b):
    return jnp.dot(a, b, preferred_element_type=F32)


def _dot_nt(a, b):
    return lax.dot_general(a, b, _NT, preferred_element_type=F32)


def _recip(x):
    return pl.reciprocal(x, approx=True)


def _upk(x):
    return pltpu.bitcast(x, BF16)


def _feature_map(s, query):
    def red(vals, op):
        a = op(op(vals[0], vals[1]), op(vals[2], vals[3]))
        a = op(a, vals[4])
        a = op(a, pltpu.roll(a, 2, 0))
        a = op(a, pltpu.roll(a, 4, 0))
        return a

    mx = red(s, jnp.maximum)
    mn = red(s, jnp.minimum)
    ep = [jnp.exp2(a - mx) for a in s]
    en = [jnp.exp2(mn - a) for a in s]
    sp = red(ep, jnp.add)
    rn = _recip(red(en, jnp.add))
    if query:
        rn = rn * sp
    else:
        rp = _recip(sp)
        ep = [a * rp for a in ep]
    return jnp.concatenate(ep + [a * rn for a in en], axis=0).astype(BF16)


def _pick(a, ncols, per):
    nr = a.shape[0] // 8
    return [a[8 * (i * nr // per):8 * (i * nr // per) + 8, 128 * j:128 * j + 128]
            for j in range(ncols) for i in range(per)]


def _kernel(x_hbm, wphi_hbm, wqkv_hbm, wo_hbm, wg_hbm, wu_hbm, wd_hbm,
            out_hbm,
            x_v, wphi_v, wqkv_v, wo_v, wblk_v, wgu3_v, wd3_v, out_v, wsems, xsems, osems, fence,
            blk_scr, wq_scr, wk32_scr, sk_scr, wk3_scr, sv_scr, wv3_scr, phiq_scr, kv_scr, a_scr,
            xa_scr, xn_scr, xo_scr, vt_scr, h_scr, hq_scr, f32_scr, sa_scr, sd_scr, a3_scr, tw_scr, to_scr,
            zero_scr):
    S, D = x_v.shape
    F = wd3_v.shape[0]
    n1 = S // TS
    n2 = S // T2
    nc = F // FC
    PH = TS // 2
    nb = PH // QB
    HR = T2 // 2

    def qkv_copy(j):
        return pltpu.make_async_copy(wqkv_hbm.at[:, pl.ds(j * D, D)], wqkv_v.at[j], wsems.at[j])

    def x_copy(t):
        return pltpu.make_async_copy(x_hbm.at[0, pl.ds(t * TS, TS), :], x_v.at[pl.ds(t * TS, TS), :], xsems.at[t])

    def out_copy(t):
        return pltpu.make_async_copy(out_v.at[pl.ds(t * T2, T2), :], out_hbm.at[0, pl.ds(t * T2, T2), :], osems.at[t])

    def part_copies(parts, sem):
        cps = []
        for p in parts:
            for u in range(2):
                if p < 6:
                    src = (wg_hbm, wu_hbm)[u].at[pl.ds(0, K2), pl.ds(p * KH, KH)]
                else:
                    src = wd_hbm.at[pl.ds((p - 6) * FC, FC), pl.ds(u * KH, KH)]
                cps.append(pltpu.make_async_copy(src, wblk_v.at[p, u], sem))
        return cps

    wphi_copy = pltpu.make_async_copy(wphi_hbm, wphi_v, wsems.at[7])
    groups = [part_copies((0,), wsems.at[4]), part_copies(range(1, 1 + NP), wsems.at[5]),
              part_copies(range(1 + NP, 1 + 2 * NP), wsems.at[6])]
    late = [pltpu.make_async_copy(wo_hbm, wo_v, wsems.at[3]),
            pltpu.make_async_copy(wg_hbm.at[pl.ds(K2, D - K2), :], wgu3_v.at[0], wsems.at[3]),
            pltpu.make_async_copy(wu_hbm.at[pl.ds(K2, D - K2), :], wgu3_v.at[1], wsems.at[3]),
            pltpu.make_async_copy(wd_hbm.at[:, pl.ds(K2, D - K2)], wd3_v, wsems.at[3])]
    late += part_copies(range(1 + 2 * NP, 9), wsems.at[3])
    slot = lambda p: ((p + NP - 1) // NP, (p + NP - 1) % NP)

    step = pl.program_id(0)
    tw_u, sa_u, sd_u, a3_u, phiq_u, wd3_u = [
        r.bitcast(U32) for r in (tw_scr, sa_scr, sd_scr, a3_scr, phiq_scr, wd3_v)]
    wq_u, sk_u, wk3_u, sv_u, wv3_u, xo_u, vt_u = [
        r.bitcast(U32) for r in (wq_scr, sk_scr, wk3_scr, sv_scr, wv3_scr, xo_scr, vt_scr)]

    def raw_tile(pb, kt):
        return 20 + 5 * pb + kt

    def x_tile(j, i, k):
        if i == 2:
            return raw_tile(j, k)
        if i == 5:
            return raw_tile(j + nb, 2 + k)
        return 10 * j + 2 * _SUMMED.index(i - 1) + k

    def ln_block(dst, base, pb):
        xn = _ln(x_v[pl.ds(base + pb * QB, QB), :].astype(F32))
        xn_scr[pb * QB:(pb + 1) * QB, :] = xn[:, 0:K2]
        for kt in range(D // 128):
            xo_scr[dst, raw_tile(pb, kt)] = xn[:, 128 * kt:128 * kt + 128].astype(BF16)
        return xn

    def x_sums(dst, j, which=_SUMMED):
        for i in which:
            for k in range(2):
                quad = lambda u: xn_scr[(u % 2) * PH + j * QB:(u % 2) * PH + (j + 1) * QB,
                                        (u // 2) * KH + 128 * k:(u // 2) * KH + 128 * k + 128]
                xo_scr[dst, x_tile(j, i + 1, k)] = _pair_sum(_RS, i, quad).astype(BF16)

    def w_sums(dst, load, h, blk):
        for r0 in range(0, h, blk):
            q = [load(h0 + r0, h0 + r0 + blk, k0, k0 + KH) for h0 in (0, h) for k0 in (0, KH)]
            for i, sv in enumerate(_lsum(*q)):
                for k in range(2):
                    dst[i, k, r0:r0 + blk, :] = sv[:, 128 * k:128 * k + 128].astype(BF16)

    @pl.when(step == 0)
    def _prologue():
        x0a = pltpu.make_async_copy(x_hbm.at[0, pl.ds(0, QB), :], x_v.at[pl.ds(0, QB), :], wsems.at[8])
        x0b = pltpu.make_async_copy(x_hbm.at[0, pl.ds(QB, TS - QB), :], x_v.at[pl.ds(QB, TS - QB), :], xsems.at[0])
        for cp in ([x0a, wphi_copy, qkv_copy(2), x0b, qkv_copy(1), qkv_copy(0)]
                   + [cp for t in range(1, n1) for cp in [x_copy(t)] + groups[t - 1]] + late):
            cp.start()
            pl.semaphore_signal(fence, 1)
            pl.semaphore_wait(fence, 1)
        kv_scr[...] = jnp.zeros_like(kv_scr)
        zero_scr[...] = jnp.zeros_like(zero_scr)
        vt_scr[:, :, :, GR:GR + 8, :] = jnp.ones((2, TS // QB, NG, 8, QB), BF16)

        fcol, _ = _row_tables(DH)
        _, hcol = _row_tables(128)
        kk = lax.broadcasted_iota(jnp.int32, (D, D), 0)
        cc = lax.broadcasted_iota(jnp.int32, (D, D), 1)
        perm = jnp.where(cc == (kk & (H - 1)) * DH + (kk >> 5), 1.0, 0.0).astype(BF16)

        def v_rows(xn, pb):
            vt = _dot(xn.astype(BF16), wqkv_v[2]).T.astype(BF16)
            for g in range(NG):
                vt_scr[0, pb, g, 0:GR, :] = vt[g * GR:(g + 1) * GR]

        x0a.wait()
        xa_scr[...] = ln_block(0, 0, 0)
        wphi_copy.wait()
        w3 = wphi_v[...].astype(F32)
        wr = jnp.concatenate([w3[d] for d in range(DH)], axis=1).astype(BF16)
        xf = _dot(wr, perm).astype(BF16)
        for t, (r0, r1) in enumerate(_RANGES):
            n = r1 - r0 + 32
            r = lax.broadcasted_iota(jnp.int32, (32, 128), 0)
            f = jnp.concatenate([jnp.zeros((32, DH), jnp.int32), fcol[r0:r1]], axis=0)
            hd = jnp.concatenate([6 * t + (r >> 3) * 2 + (r & 1), hcol[r0:r1]], axis=0)
            et = jnp.where(lax.broadcasted_iota(jnp.int32, (n, DH), 1) == f, 1.0, 0.0).astype(BF16)
            full = _dot(et, xf[:, 128 * t:128 * t + 128])
            lo = hd * DH - 128 * t
            c = lax.broadcasted_iota(jnp.int32, (n, 128), 1)
            mask = (c >= lo) & (c < lo + DH)
            blk_scr[0, t, 0:n, :] = jnp.where(mask, full, 0.0).astype(BF16)
            blk_scr[1, t, 0:n - 32, :] = jnp.where(mask[32:], (full[32:] - full[0:1]) * LOG2E, 0.0).astype(BF16)

        def fold(j, emit):
            pair = lax.broadcasted_iota(jnp.int32, (8, D), 0) >> 1
            prev, done = None, 0
            for t, (r0, r1) in enumerate(_RANGES):
                res = _dot_nt(blk_scr[j, t, 0:r1 - r0 + 32 * (1 - j), :], wqkv_v[j, :, 128 * t:128 * t + 128])
                if j == 0:
                    z = {3 * t + u: res[8 * u:8 * u + 8] for u in range(4)}
                    slabs = []
                    for nm in _ORDER:
                        g, o = int(nm[1:]), _OFF[nm] - r0 + 32
                        if not 32 <= o < r1 - r0 + 32:
                            continue
                        if nm[0] == "g":
                            slabs += [res[o + 8 * u:o + 8 * u + 8] - z[g] for u in range(4)]
                        else:
                            gg, i = _HOST[g]
                            slabs.append(res[o:o + 8] - jnp.where(pair == 3 - i, z.get(gg, 0.0), z.get(g, 0.0)))
                    res = jnp.concatenate(slabs, axis=0) * LOG2E
                if prev is not None:
                    a, b = r0 - done, prev.shape[0] - (r0 - done)
                    res = jnp.concatenate(([prev[0:a]] if a else []) + [res[0:b] + prev[a:], res[b:]], axis=0)
                end = _RANGES[t + 1][0] // 16 * 16 if t < 4 else r1
                emit(done, res[0:end - done])
                prev = res[end - done:] if t < 4 else None
                done = end

        def emit_k(r0, w):
            wk32_scr[r0:r0 + w.shape[0], :] = w[:, 0:K2]
            wk3_scr[r0:r0 + w.shape[0], :] = w[:, K2:].astype(BF16)

        def emit_q(r0, w):
            for kt in range(D // 128):
                wq_scr[kt, r0:r0 + w.shape[0], :] = w[:, 128 * kt:128 * kt + 128].astype(BF16)

        qkv_copy(2).wait()
        v_rows(xa_scr[...], 0)
        x0b.wait()
        xs = [ln_block(0, 0, pb) for pb in range(1, TS // QB)]
        wvt = wqkv_v[2].T
        w_sums(sv_scr, lambda r0, r1, c0, c1: wvt[r0:r1, c0:c1].astype(F32), D // 2, 32)
        wv3_scr[...] = wvt[:, K2:]
        for pb in range(1, TS // QB):
            v_rows(xs[pb - 1], pb)
        for j in range(nb):
            x_sums(0, j)
        qkv_copy(0).wait()
        qkv_copy(1).wait()
        fold(1, emit_k)
        fold(0, emit_q)
        w_sums(sk_scr, lambda r0, r1, c0, c1: wk32_scr[r0:r1, c0:c1], PR // 2, 16)

    def fmaps(pt, groups, query=False):
        base = (groups[0] // 4) * (PR // 4)
        return [_feature_map(_group_slabs(pt, g, base), query) for g in groups]

    def kv_update(phik, cur, which):
        for g in range(NG):
            acc = kv_scr[g]
            for j in sorted(which):
                acc = acc + _dot_nt(_upk(vt_u[cur, j, g]), phik[j][g])
            kv_scr[g] = acc

    def product(s_u, buf, j, i):
        return sum(_dot_nt(_upk(s_u[i - 1, k]), _upk(xo_u[buf, x_tile(j, i, k)])) for k in range(2))

    def quadrant(name, M, w3_u, buf, j):
        rh, ph = int(name[0]) - 1, int(name[1]) - 1
        h = w3_u.shape[0] // 2
        r = _dot_nt(_upk(w3_u[rh * h:(rh + 1) * h, :]), _upk(xo_u[buf, raw_tile(ph * nb + j, 4)]))
        if name == "21":
            return M[2] + M[4] + r
        if name == "12":
            return M[3] + M[5] + r
        if name == "11":
            return (M[4] - M[5] + M[1]) + M[7] + r
        return (M[3] - M[2] + M[1]) + M[6] + r

    def weight_prep(parts, ys):
        blocks = []
        for p in parts:
            if p is None:
                blocks += [(p, r0, 0) for r0 in range(0, KH, PB)]
            else:
                blocks += [(p, r0, i) for i in range(7) for r0 in range(0, 128, PB)]
        for bi, (part, r0, i) in enumerate(blocks):
            y = ys[bi * len(ys) // len(blocks)]
            z = pltpu.bitcast(pltpu.bitcast(y, U32) & zero_scr[...], F32)
            z = jnp.concatenate([z] * (PB // 8), axis=0)
            if part is None:
                q = [wo_v[k0 + r0:k0 + r0 + PB, n0:n0 + KH].astype(F32) for k0 in (0, KH) for n0 in (0, KH)]
                z = jnp.concatenate([z, z], axis=1)
                tv = _rsum(q[0] + z, q[1], q[2], q[3] + z)
                for k, p in enumerate(_SUMMED):
                    to_scr[k, r0:r0 + PB, :] = tv[p].astype(BF16)
                continue

            def src(qi):
                k0 = (qi // 2) * KH + r0
                return jnp.concatenate(
                    [wblk_v[part[0], qi % 2, k0 + d:k0 + d + PB, :].astype(F32) for d in (0, 128)], axis=0)

            b11, b12, b21, b22 = _quads(_pair_sum(_RS, i, src))
            for j, s2 in enumerate(_rsum(b11 + z, b12, b21, b22 + z)):
                tw_scr[part[1], part[2], 7 * i + j, r0:r0 + PB, :] = s2.astype(BF16)

    def qk_token(tok, t, cur, st, phik, taps):
        if tok[:2] == "kv":
            kv_update(phik, cur, [int(c) for c in tok[2:]])
        elif tok[0] == "q":
            pb = int(tok[1])
            parts = [_dot_nt(_upk(wq_u[kt]), _upk(xo_u[cur, raw_tile(pb, kt)])) for kt in range(D // 128)]
            taps["q"].append(parts[0])
            for g, ph in enumerate(fmaps(sum(parts), range(NG), True)):
                phiq_scr[t * 2 * nb + pb, g * 2 * GR:(g + 1) * 2 * GR, :] = ph
        else:
            j = "ab".index(tok[0])
            M = st.setdefault(("M", j), {})
            if len(tok) == 2:
                M[int(tok[1])] = product(sk_u, cur, j, int(tok[1]))
                taps["k"].append(M[int(tok[1])])
            else:
                g0, ph = (int(tok[1]) - 1) * (NG // 2), int(tok[2]) - 1
                gs = range(g0, g0 + NG // 2)
                for g, f in zip(gs, fmaps(quadrant(tok[1:], M, wk3_u, cur, j), gs)):
                    phik[ph * nb + j][g] = f

    @pl.when(jnp.logical_and(step >= 1, step < n1))
    def _p1():
        t = step - 1
        cur = t % 2
        nxt = 1 - cur
        x_copy(t + 1).wait()
        for k in range(n1 - 1):
            @pl.when(t == k)
            def _():
                for cp in groups[k]:
                    cp.wait()

        phik = [[None] * NG for _ in range(2 * nb)]
        st = {}
        taps = dict(q=[], k=[], v=[])
        base = pl.multiple_of((t + 1) * TS, TS)
        for tok in _SCRIPT1.split():
            if tok[0] != "V":
                qk_token(tok, t, cur, st, phik, taps)
                continue
            j = "ab".index(tok[1])
            M = {}
            for op in _V_ORDER.split():
                if op[0] == "L":
                    ln_block(nxt, base, int(op[1]) * nb + j)
                elif op[0] == "s":
                    x_sums(nxt, j, [int(c) - 1 for c in op[1:]])
                elif op[0] == "c":
                    v = quadrant(op[1:], M, wv3_u, nxt, j)
                    g0, ph = (int(op[1]) - 1) * (NG // 2), int(op[2]) - 1
                    for g in range(NG // 2):
                        vt_scr[nxt, ph * nb + j, g0 + g, 0:GR, :] = v[g * GR:(g + 1) * GR].astype(BF16)
                else:
                    M[int(op)] = product(sv_u, nxt, j, int(op))
                    taps["v"].append(M[int(op)])
        ys = ([y for m in taps["q"] for y in _pick(m, 1, _PINS1[0])] + _pick(taps["k"][0], 1, _PINS1[4])
              + [y for m in taps["k"][1:] for y in _pick(m, 1, _PINS1[1])]
              + [y for m in taps["v"][0:7] for y in _pick(m, 1, _PINS1[2])]
              + [y for m in taps["v"][7:13] for y in _pick(m, 1, _PINS1[3])])
        weight_prep([(jnp.maximum(NP * (t - 1) + 1 + k, 0), t, k) for k in range(NP)], ys)

    def attn_num_den(blk):
        return [_dot(a_scr[g], _upk(phiq_u[blk, g * GR:(g + 1) * GR, :])) for g in range(NG)]

    def normalize(res):
        sub = lax.broadcasted_iota(jnp.int32, (8, res[0].shape[1]), 0) < 4
        pieces = []
        for oe in res:
            r = _recip(oe[40:48])
            rr = pltpu.roll(r, 4, 0)
            ra = jnp.where(sub, r, rr)
            rb = jnp.where(sub, rr, r)
            pieces += [oe[0:8] * ra, oe[8:16] * ra, oe[16:24] * r, oe[24:32] * rb, oe[32:40] * rb]
        return jnp.concatenate(pieces, axis=0)

    def out_proj(res):
        ot = normalize(res)
        o = ot.T.astype(BF16)
        a11, a12, a21, a22 = ot[0:KH, 0:HR], ot[KH:K2, 0:HR], ot[0:KH, HR:], ot[KH:K2, HR:]
        tr = lambda a: a.T.astype(BF16)
        r3 = _dot(o, wo_v[:, K2:])
        rk = _dot(o[:, K2:], wo_v[K2:, 0:K2])
        m1 = _dot(tr(a11 + a22), to_scr[0])
        m4 = _dot(o[HR:, KH:K2], to_scr[2])
        m5 = _dot(tr(a11 + a12), wo_v[KH:K2, KH:K2])
        m7 = _dot(tr(a12 - a22), to_scr[4])
        m3 = _dot(o[0:HR, 0:KH], to_scr[1])
        m2 = _dot(tr(a21 + a22), wo_v[0:KH, 0:KH])
        m6 = _dot(tr(a21 - a11), to_scr[3])
        top = jnp.concatenate([m1 + m4 - m5 + m7, m3 + m5], axis=1)
        bot = jnp.concatenate([m2 + m4, m1 - m2 + m3 + m6], axis=1)
        return jnp.concatenate([jnp.concatenate([top, bot], axis=0) + rk, r3], axis=1)

    def store49(dst, src):
        q = HR // 2
        for i in (4, 2, 5, 3, 1, 7, 6):
            for r0 in range(0, q, PB):
                quad = lambda u: jnp.concatenate(
                    [src[(u // 2) * HR + d + r0:(u // 2) * HR + d + r0 + PB, (u % 2) * KH:(u % 2 + 1) * KH]
                     for d in (0, q)], axis=0)
                for j, s2 in enumerate(_lsum(*_quads(_pair_sum(_LS, i - 1, quad)))):
                    dst[7 * (i - 1) + j, r0:r0 + PB, :] = s2.astype(BF16)

    def load_sa():
        return [[_upk(sa_u[7 * i + j]) for j in range(7)] for i in range(7)], _upk(a3_u[...])

    def residual_ln2(t, attn):
        hq_scr[...] = x_v[pl.ds(pl.multiple_of(t * T2, T2), T2), :].astype(F32) + attn
        hn = _ln(hq_scr[...])
        a3_scr[...] = hn[:, K2:].astype(BF16)
        f32_scr[nc] = hn[:, 0:K2]
        store49(sa_scr, f32_scr.at[nc])
        return (hq_scr[...],) + load_sa()

    def gate_up(sa, a3, c, order=_GU_ORDER[0]):
        a1, a2 = [], []
        for b in range(c * FC // KH, (c + 1) * FC // KH):
            m = lambda i: _comb(lambda j: _dot(sa[i - 1][j - 1], _upk(tw_u[slot(b) + (7 * (i - 1) + j - 1,)])))
            P = {}
            for k in order:
                P[k] = _dot(a3, wgu3_v["gu".index(k), :, b * KH:(b + 1) * KH]) if k in "gu" else m(int(k))
            m1, m2, m3, m4, m5, m6, m7, rg, ru = [P[k] for k in "1234567gu"]
            g2 = m2 + m4 + rg[HR:]
            u1 = m3 + m5 + ru[0:HR]
            g1 = (m4 - m5 + rg[0:HR]) + (m1 + m7)
            u2 = (m3 - m2 + ru[HR:]) + (m1 + m6)
            a1.append(_geglu2(g1, u1))
            a2.append(_geglu2(g2, u2))
        return jnp.concatenate(a1, axis=1), jnp.concatenate(a2, axis=1), c

    def down(acts, order=None):
        for a1, a2, c in acts:
            f32_scr[c, 0:HR, :] = a1
            f32_scr[c, HR:, :] = a2
            store49(sd_scr.at[c], f32_scr.at[c])
        sd = [[[_upk(sd_u[c, 7 * i + j]) for j in range(7)] for i in range(7)] for a1, a2, c in acts]
        r3 = sum(_dot(jnp.concatenate([a1, a2], axis=0).astype(BF16), _upk(wd3_u[c * FC // 2:(c + 1) * FC // 2, :]))
                 for a1, a2, c in acts)
        m = lambda i: _comb(
            lambda j: sum(_dot(sd[k][i - 1][j - 1], _upk(tw_u[slot(6 + acts[k][2]) + (7 * (i - 1) + j - 1,)]))
                          for k in range(len(acts))), order)
        return 0.5 * jnp.concatenate([_comb(m, order), r3], axis=1)

    @pl.when(step == n1)
    def _trans():
        for cp in late:
            cp.wait()
        t = n1 - 1
        phik = [[None] * NG for _ in range(2 * nb)]
        st = {}
        taps = dict(q=[], k=[])
        for tok in _SCRIPT2.split():
            if tok == "Mid":
                r = lax.broadcasted_iota(jnp.int32, (48, 2 * GR), 0)
                c = lax.broadcasted_iota(jnp.int32, (48, 2 * GR), 1)
                hr = jnp.where(r < 40, (r >= DH).astype(jnp.int32), (r >= 44).astype(jnp.int32))
                mask = hr == (c & 1)
                eps = jnp.where((r >= 40) & (c < GR), 1e-6, 0.0)
                for g in range(NG):
                    a_scr[g] = jnp.where(mask, kv_scr[g] + eps, 0.0).astype(BF16)
            elif tok[0] == "o":
                st[tok] = attn_num_den(int(tok[1]))
            elif tok[0] == "w":
                st[tok] = _dot(normalize(st["o" + tok[1]]).T.astype(BF16), wo_v[...])
            elif tok == "ffn":
                h, sa, a3 = residual_ln2(0, jnp.concatenate([st["w%d" % j] for j in range(nb)], axis=0))
                h_scr[...] = h + down([gate_up(sa, a3, 0, _GU_ORDER[1])])
            else:
                qk_token(tok, t, t % 2, st, phik, taps)
        ys = ([y for m in taps["q"] for y in _pick(m, 1, _PINS2[0])] + _pick(taps["k"][0], 1, _PINS2[3])
              + [y for m in taps["k"][1:] for y in _pick(m, 1, _PINS2[1])]
              + [y for j in range(nb) for y in _pick(st["w%d" % j], 4, _PINS2[2])])
        weight_prep([None] + [(p,) + slot(p) for p in range(1 + 2 * NP, 9)], ys)

    @pl.when(jnp.logical_and(step > n1, step < n1 + n2))
    def _p2():
        t = step - n1 - 1
        sa, a3 = load_sa()
        res = [jnp.concatenate([_dot(a_scr[g], _upk(phiq_u[(t + 1) * nb + j, g * GR:(g + 1) * GR, :]))
                                for j in range(nb)], axis=1) for g in range(NG)]
        acts = [gate_up(sa, a3, c) for c in range(1, nc)]
        attn = out_proj(res)
        out_v[pl.ds(pl.multiple_of(t * T2, T2), T2), :] = (h_scr[...] + down(acts)).astype(out_v.dtype)
        out_copy(t).start()
        h, sa, a3 = residual_ln2(t + 1, attn)
        h_scr[...] = h + down([gate_up(sa, a3, 0)])

    @pl.when(step == n1 + n2)
    def _last():
        sa, a3 = load_sa()
        o = h_scr[...] + down([gate_up(sa, a3, c, _GU_ORDER[2]) for c in range(1, nc)], _LAST_ORDER)
        base = (n2 - 1) * T2
        tails = []
        for i, (r0, r1, c0, c1) in enumerate(_LAST_SPLIT):
            out_v[base + r0:base + r1, c0:c1] = o[r0:r1, c0:c1].astype(out_v.dtype)
            cp = pltpu.make_async_copy(out_v.at[pl.ds(base + r0, r1 - r0), pl.ds(c0, c1 - c0)],
                                       out_hbm.at[0, pl.ds(base + r0, r1 - r0), pl.ds(c0, c1 - c0)],
                                       osems.at[n2 - 1 + i])
            cp.start()
            tails.append(cp)
        for t in range(n2 - 1):
            out_copy(t).wait()
        for cp in tails:
            cp.wait()


def _impl(A_x, A_wqkv, A_w_phi, A_wo, B_x, B_w_gate, B_w_up, B_w_down):
    B, S, D = A_x.shape
    F = B_w_gate.shape[-1]
    assert (B, S, D, F) == (1, 2048, H * DH, 1536)
    anyspec = pl.BlockSpec(memory_space=pl.ANY)
    return pl.pallas_call(
        _kernel,
        grid=(S // TS + S // T2 + 1,),
        in_specs=[anyspec] * 7,
        out_specs=anyspec,
        out_shape=jax.ShapeDtypeStruct((B, S, D), A_x.dtype),
        scratch_shapes=[
            pltpu.VMEM((S, D), BF16),
            pltpu.VMEM((DH, DH, H), BF16),
            pltpu.VMEM((3, D, D), BF16),
            pltpu.VMEM((D, D), BF16),
            pltpu.VMEM((9, 2, K2, KH), BF16),
            pltpu.VMEM((2, D - K2, F), BF16),
            pltpu.VMEM((F, D - K2), BF16),
            pltpu.VMEM((S, D), BF16),
            pltpu.SemaphoreType.DMA((9,)),
            pltpu.SemaphoreType.DMA((S // TS,)),
            pltpu.SemaphoreType.DMA((S // T2 - 1 + len(_LAST_SPLIT),)),
            pltpu.SemaphoreType.REGULAR,
            pltpu.VMEM((2, 5, 208, 128), BF16),
            pltpu.VMEM((D // 128, PR, 128), BF16),
            pltpu.VMEM((PR, K2), F32),
            pltpu.VMEM((7, 2, PR // 2, 128), BF16),
            pltpu.VMEM((PR, D - K2), BF16),
            pltpu.VMEM((7, 2, D // 2, 128), BF16),
            pltpu.VMEM((D, D - K2), BF16),
            pltpu.VMEM((S // QB, 2 * D, QB), BF16),
            pltpu.VMEM((NG, 48, 2 * GR), F32),
            pltpu.VMEM((NG, 48, 2 * GR), BF16),
            pltpu.VMEM((QB, D), F32),
            pltpu.VMEM((TS, K2), F32),
            pltpu.VMEM((2, 40, 128, 128), BF16),
            pltpu.VMEM((2, TS // QB, NG, 48, QB), BF16),
            pltpu.VMEM((T2, D), F32),
            pltpu.VMEM((T2, D), F32),
            pltpu.VMEM((F // FC + 1, T2, K2), F32),
            pltpu.VMEM((49, T2 // 4, 128), BF16),
            pltpu.VMEM((F // FC, 49, T2 // 4, 128), BF16),
            pltpu.VMEM((T2, D - K2), BF16),
            pltpu.VMEM((4, NP, 49, 128, 128), BF16),
            pltpu.VMEM((5, KH, KH), BF16),
            pltpu.VMEM((8, 128), U32),
        ],
        compiler_params=pltpu.CompilerParams(
            dimension_semantics=("arbitrary",),
            vmem_limit_bytes=100 * 1024 * 1024,
            disable_bounds_checks=True,
            disable_semaphore_checks=True,
        ),
    )(A_x, jnp.transpose(A_w_phi, (1, 2, 0)), A_wqkv, A_wo, B_w_gate, B_w_up, B_w_down)


@jax.jit
def pallas_sequential_preLN__linear_kernel_hedgehog__geglu_ffn__prompt_kernel(
        A_x, A_wqkv, A_w_phi, A_wo, B_x, B_w_gate, B_w_up, B_w_down):
    return _impl(A_x, A_wqkv, A_w_phi, A_wo, B_x, B_w_gate, B_w_up, B_w_down)
```
